```python
import os as _os
_os.environ.setdefault("JAX_PLATFORMS", "cpu")
import jax
import jax.numpy as jnp

def _softmax(x, axis=-1):
    return jax.nn.softmax(x, axis=axis)
def _gelu(x):
    return jax.nn.gelu(x, approximate=True)
def _silu(x):
    return jax.nn.silu(x)
def _sigmoid(x):
    return jax.nn.sigmoid(x)
def _layernorm(x, axis=-1, eps=1e-5):
    m = jnp.mean(x, axis=axis, keepdims=True)
    v = jnp.var(x, axis=axis, keepdims=True)
    return (x - m) / jnp.sqrt(v + eps)
def _scatter_add(tgt, idx, src, axis=0):
    return tgt.at[idx].add(src)
def _segment_sum(src, seg, n):
    return jax.ops.segment_sum(src, seg, n)
class _Rng:
    def __init__(self, key):
        self._k = key
    def _next(self):
        self._k, sub = jax.random.split(self._k)
        return sub
    def normal(self, shape):
        return jax.random.normal(self._next(), shape, dtype=jnp.bfloat16)
    def randint(self, lo, hi, shape):
        return jax.random.randint(self._next(), shape, lo, hi, dtype=jnp.int32)
    def uniform(self, shape, lo=0.0, hi=1.0):
        return jax.random.uniform(self._next(), shape, jnp.bfloat16, lo, hi)
    def permutation(self, n):
        return jax.random.permutation(self._next(), n)


kernel_name = 'gated_mix__mha_block_cached__swiglu_ffn__decode'

def setup_inputs():
    _rng = _Rng(jax.random.key(int.from_bytes(__import__("os").urandom(4), "little")))
    _w = (lambda a: (lambda t: t.astype(jnp.bfloat16) if jnp.issubdtype(t.dtype, jnp.floating) else t)(jnp.asarray(a)))
    def _A_setup():
        B, Sq, D = 4, 1, 512
        H, Sk, Dh = 32, 4096, 128
        return {
            "x": _w((lambda *s: _rng.normal(s) * 0.05)(B, Sq, D)),
            "k_cache": _w((lambda *s: _rng.normal(s) * 3.2)(B, H, Sk, Dh)),
            "v_cache": _w((lambda *s: _rng.normal(s) * 0.4)(B, H, Sk, Dh)),
            "wq": _w((lambda *s: _rng.normal(s) * 3.2)(D, H * Dh) * (D ** -0.5)),
            "wo": _w((lambda *s: _rng.normal(s) * 0.4)(H * Dh, D) * ((H * Dh) ** -0.5)),
        }
    _A_in = _A_setup()

    def _B_setup():
        B, S, D, F = 4, 1, 512, 1376
        return {
            "x": _w((lambda *s: _rng.normal(s) * 0.05)(B, S, D)),
            "w_gate": _w((lambda *s: _rng.normal(s) * 0.05)(D, F)),
            "w_up": _w((lambda *s: _rng.normal(s) * 0.05)(D, F)),
            "w_down": _w((lambda *s: _rng.normal(s) * 0.05)(F, D)),
        }
    _B_in = _B_setup()

    return {
        "A_x": _A_in["x"],
        "A_k_cache": _A_in["k_cache"],
        "A_v_cache": _A_in["v_cache"],
        "A_wq": _A_in["wq"],
        "A_wo": _A_in["wo"],
        "B_x": _B_in["x"],
        "B_w_gate": _B_in["w_gate"],
        "B_w_up": _B_in["w_up"],
        "B_w_down": _B_in["w_down"],
        "gate_w": _w((lambda *s: _rng.normal(s) * 0.05)(512) * 16.0),
    }

def reference(A_x, A_k_cache, A_v_cache, A_wq, A_wo, B_x, B_w_gate, B_w_up, B_w_down, gate_w):
    def _A_ref(x, k_cache, v_cache, wq, wo):
        B, Sq, D = x.shape
        H, Dh = 32, 128
        q = (lambda x, *d: x.transpose(*d))((x @ wq).reshape(B, Sq, H, Dh), 0, 2, 1, 3)
        scores = jnp.einsum("bhqd,bhkd->bhqk", q, k_cache) * (Dh ** -0.5)
        p = _softmax(scores, axis=-1)
        o = jnp.einsum("bhqk,bhkd->bhqd", p, v_cache)
        return (lambda x, *d: x.transpose(*d))(o, 0, 2, 1, 3).reshape(B, Sq, H * Dh) @ wo

    def _B_ref(x, w_gate, w_up, w_down):
        g = _silu(x @ w_gate)
        u = x @ w_up
        return (g * u) @ w_down

    x = A_x
    g = _sigmoid((x * gate_w).sum(-1, keepdims=True))
    a = _A_ref(x, A_k_cache, A_v_cache, A_wq, A_wo)
    b = _B_ref(x, B_w_gate, B_w_up, B_w_down)
    return g * a + (1 - g) * b
```

```python
import jax
import jax.numpy as jnp
from jax import lax
import jax.experimental.pallas as pl
import jax.experimental.pallas.tpu as pltpu

T = 128
NS = 8
WROWS = 32
QROWS = 8


def _nt_dot(a, b):
    return lax.dot_general(a, b, (((1,), (1,)), ((), ())), preferred_element_type=jnp.float32)


def _dot(a, b):
    return jnp.dot(a, b, preferred_element_type=jnp.float32)


def make_kernel(B, D, H, SK, DH, F, *, ahead=6, ring=8):
    NKC = SK // T
    NG = B * H // NS
    NT = NG * NKC
    HB = H // NG
    QCOLS = T * DH // QROWS
    QCPR = (H * DH) // QCOLS
    NA = (D // QROWS) * QCPR // (2 * NS)
    NFB = pl.cdiv(F, T)
    FU = F // WROWS
    FR = FU - NKC
    scale = DH ** -0.5
    assert ahead <= NA and ahead < ring

    def kernel(x_hbm, gw_hbm, k_hbm, v_hbm, wq_hbm, wo_hbm, wg_hbm, wu_hbm, wd_hbm, o_ref,
               kv_buf, wq_buf, wo_buf, wg_buf, wu_buf, wd_buf, x_buf, gw_buf, s_buf, y_buf, f_buf,
               sem, misc_sem):
        ffn = ((wg_hbm, wg_buf), (wu_hbm, wu_buf), (wd_hbm, wd_buf))

        def start(c, q):
            c.start(priority=q)

        def wait(c, q):
            c.wait()

        def tile(hbm, t, s, slot, q):
            return pltpu.make_async_copy(
                hbm.at[s, pl.ds(pl.multiple_of(t * T, T), T)], kv_buf.at[slot, s, q], sem.at[slot])

        def rows(hbm, buf, u, sm):
            r = pl.ds(pl.multiple_of(u * WROWS, WROWS), WROWS)
            return pltpu.make_async_copy(hbm.at[r], buf.at[r], sm)

        def wq_pair(a, s, op):
            for q in range(2):
                u = (2 * s + q) * NA + a
                r = pl.ds(pl.multiple_of((u // QCPR) * QROWS, QROWS), QROWS)
                c = pl.ds(pl.multiple_of((u % QCPR) * QCOLS, QCOLS), QCOLS)
                op(pltpu.make_async_copy(wq_hbm.at[r, c], wq_buf.at[r, c], sem.at[a % ring]), q)

        def first_pair(g, s, op):
            slot = (g + NA) % ring
            sm = sem.at[slot]
            for q in range(2):
                if q == 0:
                    op(tile(k_hbm, g, s, slot, 0), 0)
                elif s < 4:
                    op(rows(wo_hbm, wo_buf, s * NKC + g, sm), 1)
                elif s < 7:
                    op(rows(*ffn[s - 4], g, sm), 1)
                elif isinstance(g, int):
                    op(rows(*ffn[g // FR], NKC + g % FR, sm), 1)
                else:
                    for j in range(3):
                        @pl.when(g // FR == j)
                        def _():
                            op(rows(*ffn[j], NKC + g - j * FR, sm), 1)

        def main_pair(g, s, op):
            slot = (g + NA) % ring
            for q in range(2):
                op(tile(k_hbm, g, s, slot, 0) if q == 0 else tile(v_hbm, g - NKC, s, slot, 1), q)

        def last_pair(j, s, op):
            slot = (j + NT + NA) % ring
            for q in range(2):
                op(tile(v_hbm, NT - NKC + j + q * (NKC // 2), s, slot, q), q)

        def wait_slot(slot):
            wait(pltpu.make_async_copy(kv_buf.at[slot], kv_buf.at[slot], sem.at[slot]), 0)

        row = lax.broadcasted_iota(jnp.int32, (NS, DH), 0)

        small = [pltpu.make_async_copy(x_hbm, x_buf, misc_sem.at[0]),
                 pltpu.make_async_copy(gw_hbm, gw_buf, misc_sem.at[1]),
                 rows(wd_hbm, wd_buf, FU - 1, misc_sem.at[2])]

        @pl.loop(0, ahead)
        def _(a):
            for s in range(NS):
                wq_pair(a, s, start)

        for c in small:
            start(c, 0)

        if ahead < NA:
            @pl.loop(0, NA - ahead)
            def _(a):
                for s in range(NS):
                    wq_pair(a, s, wait)
                for s in range(NS):
                    wq_pair(a + ahead, s, start)

        @pl.loop(NA - ahead, NA)
        def _(a):
            for s in range(NS):
                wq_pair(a, s, wait)
            for s in range(NS):
                first_pair(a + ahead - NA, s, start)

        for c in small:
            wait(c, 0)
        xf = x_buf[...].astype(jnp.float32)
        row_d = lax.broadcasted_iota(jnp.int32, (NS, D), 0)
        x8f = jnp.zeros((NS, D), jnp.float32)
        for b in range(B):
            x8f = jnp.where(row_d // HB == b, xf[b:b + 1, :], x8f)
        x8 = x8f.astype(jnp.bfloat16)

        def q_proj(i):
            q = jnp.zeros((NS, DH), jnp.float32)
            for hh in range(HB):
                c = pl.ds(pl.multiple_of((hh * NG + i) * DH, DH), DH)
                q = jnp.where(row % HB == hh, _dot(x8, wq_buf[:, c]), q)
            return q.astype(jnp.bfloat16)

        def out_proj(i, acc, l):
            o = acc / jnp.sum(l, axis=1, keepdims=True)
            y = y_buf[...]
            for hh in range(HB):
                r = pl.ds(pl.multiple_of((hh * NG + i) * DH, DH), DH)
                y += _dot(jnp.where(row % HB == hh, o, 0.0).astype(jnp.bfloat16), wo_buf[r, :])
            y_buf[...] = y

        def ffn_block(f):
            r0 = jnp.minimum(f * T, F - T)
            r = pl.ds(pl.multiple_of(r0, WROWS), T)
            g = _nt_dot(x8, wg_buf[r, :])
            u = _nt_dot(x8, wu_buf[r, :])
            h = g * jax.nn.sigmoid(g) * u
            col = lax.broadcasted_iota(jnp.int32, (NS, T), 1)
            h = jnp.where(col + r0 >= f * T, h, 0.0)
            f_buf[...] += _dot(h.astype(jnp.bfloat16), wd_buf[r, :])

        y_buf[...] = jnp.zeros_like(y_buf)
        f_buf[...] = jnp.zeros_like(f_buf)
        neg_inf = jnp.full((NS, T), -jnp.inf, jnp.float32)
        zeros = jnp.zeros((NS, T), jnp.float32)

        def first_step(g, q, mx, next_pair):
            slot = (g + NA) % ring
            for s in range(NS):
                first_pair(g, s, wait)
            sc = zeros
            for s in range(NS):
                next_pair(g + ahead, s, start)
                sc = jnp.where(row == s, _nt_dot(q, kv_buf[slot, s, 0]), sc)
            sc = sc * scale
            s_buf[g] = sc
            return jnp.maximum(mx, sc)

        q = q_proj(0)
        mx = lax.fori_loop(0, NKC - ahead, lambda g, mx: first_step(g, q, mx, first_pair), neg_inf)
        mx = lax.fori_loop(NKC - ahead, NKC, lambda g, mx: first_step(g, q, mx, main_pair), mx)

        def main_step(g, carry, start_next):
            q, m, mx, l, acc = carry
            slot = (g + NA) % ring
            kc = g % NKC
            p = jnp.exp(s_buf[kc] - m)
            pb = p.astype(jnp.bfloat16)
            wait_slot(slot)
            sc = zeros
            pv = zeros
            for s in range(NS):
                start_next(s)
                sc = jnp.where(row == s, _nt_dot(q, kv_buf[slot, s, 0]), sc)
                pv = jnp.where(row == s, _dot(pb, kv_buf[slot, s, 1]), pv)
            sc = sc * scale
            s_buf[kc] = sc
            return q, m, jnp.maximum(mx, sc), l + p, acc + pv

        def row_max(mx):
            return jnp.broadcast_to(jnp.max(mx, axis=1, keepdims=True), (NS, T))

        def group(i, carry):
            mx, l, acc = carry[2:]

            @pl.when(i >= 2)
            def _():
                out_proj(i - 2, acc, l)

            @pl.when(i <= NFB)
            def _():
                ffn_block(i - 1)

            carry = (q_proj(i), row_max(mx), neg_inf, zeros, zeros)
            stop = jnp.minimum((i + 1) * NKC, NT - ahead)
            return lax.fori_loop(
                i * NKC, stop,
                lambda g, c: main_step(g, c, lambda s: main_pair(g + ahead, s, start)), carry)

        carry = lax.fori_loop(1, NG, group, (q, zeros, mx, zeros, zeros))
        carry = lax.fori_loop(
            NT - ahead, NT,
            lambda g, c: main_step(g, c, lambda s: last_pair(g + ahead - NT, s, start)), carry)
        _, _, mx, l, acc = carry
        out_proj(NG - 2, acc, l)
        m = row_max(mx)

        def last_step(j, carry, start_next):
            l, acc = carry
            slot = (j + NT + NA) % ring
            p0 = jnp.exp(s_buf[j] - m)
            p1 = jnp.exp(s_buf[j + NKC // 2] - m)
            pb0 = p0.astype(jnp.bfloat16)
            pb1 = p1.astype(jnp.bfloat16)
            wait_slot(slot)
            pv0 = zeros
            pv1 = zeros
            for s in range(NS):
                start_next(s)
                pv0 = jnp.where(row == s, _dot(pb0, kv_buf[slot, s, 0]), pv0)
                pv1 = jnp.where(row == s, _dot(pb1, kv_buf[slot, s, 1]), pv1)
            return l + (p0 + p1), acc + (pv0 + pv1)

        carry = lax.fori_loop(
            0, NKC // 2 - ahead,
            lambda j, c: last_step(j, c, lambda s: last_pair(j + ahead, s, start)), (zeros, zeros))
        l, acc = lax.fori_loop(
            NKC // 2 - ahead, NKC // 2, lambda j, c: last_step(j, c, lambda s: None), carry)
        out_proj(NG - 1, acc, l)

        gwf = gw_buf[...].astype(jnp.float32)
        z = jnp.zeros((NS, DH), jnp.float32)
        for j in range(D // DH):
            z += x8f[:, j * DH:(j + 1) * DH] * gwf[j:j + 1, :]
        gate = jax.nn.sigmoid(jnp.sum(z, axis=1, keepdims=True))
        y = y_buf[...]
        fo = f_buf[...]
        row_o = lax.broadcasted_iota(jnp.int32, (B, D), 0)
        out = jnp.zeros((B, D), jnp.float32)
        for b in range(B):
            a = y[HB * b:HB * b + 1]
            for hh in range(1, HB):
                a = a + y[HB * b + hh:HB * b + hh + 1]
            gb = gate[HB * b:HB * b + 1]
            out = jnp.where(row_o == b, gb * a + (1.0 - gb) * fo[HB * b:HB * b + 1], out)
        o_ref[...] = out.astype(o_ref.dtype)

    bf = jnp.bfloat16
    scratch = [
        pltpu.VMEM((ring, NS, 2, T, DH), bf),
        pltpu.VMEM((D, H * DH), bf),
        pltpu.VMEM((H * DH, D), bf),
        pltpu.VMEM((F, D), bf),
        pltpu.VMEM((F, D), bf),
        pltpu.VMEM((F, D), bf),
        pltpu.VMEM((B, D), bf),
        pltpu.VMEM((D // DH, DH), bf),
        pltpu.VMEM((NKC, NS, T), jnp.float32),
        pltpu.VMEM((NS, D), jnp.float32),
        pltpu.VMEM((NS, D), jnp.float32),
        pltpu.SemaphoreType.DMA((ring,)),
        pltpu.SemaphoreType.DMA((3,)),
    ]
    return kernel, scratch


@jax.jit
def pallas_gated_mix__mha_block_cached__swiglu_ffn__decode_kernel(
    A_x: jax.Array,
    A_k_cache: jax.Array,
    A_v_cache: jax.Array,
    A_wq: jax.Array,
    A_wo: jax.Array,
    B_x: jax.Array,
    B_w_gate: jax.Array,
    B_w_up: jax.Array,
    B_w_down: jax.Array,
    gate_w: jax.Array,
):
    del B_x
    B, _, D = A_x.shape
    _, H, SK, DH = A_k_cache.shape
    F = B_w_gate.shape[1]
    kernel, scratch = make_kernel(B, D, H, SK, DH, F)
    out = pl.pallas_call(
        kernel,
        out_shape=jax.ShapeDtypeStruct((B, D), A_x.dtype),
        in_specs=[pl.BlockSpec(memory_space=pl.ANY)] * 9,
        out_specs=pl.BlockSpec(memory_space=pltpu.VMEM),
        scratch_shapes=scratch,
        compiler_params=pltpu.CompilerParams(vmem_limit_bytes=48 * 2**20),
        name="gated_mix_decode",
    )(
        A_x.reshape(B, D), gate_w.reshape(D // DH, DH),
        A_k_cache.reshape(NS, B * H * SK // NS, DH), A_v_cache.reshape(NS, B * H * SK // NS, DH),
        A_wq, A_wo, B_w_gate.T, B_w_up.T, B_w_down,
    )
    return out.reshape(B, 1, D)
```

```python
import jax
import jax.numpy as jnp
from jax import lax
import jax.experimental.pallas as pl
import jax.experimental.pallas.tpu as pltpu

TILE = 128
STREAMS = 8
W_ROWS = 32
Q_ROWS = 8
AHEAD = 5
RING = 8
STAGES = (3, 1)


def _dot(a, b):
    return jnp.dot(a, b, preferred_element_type=jnp.float32)


def _dot_t(a, b):
    return lax.dot_general(a, b, (((1,), (1,)), ((), ())), preferred_element_type=jnp.float32)


def _div(a, n):
    return a // n if isinstance(a, int) else lax.shift_right_logical(a, n.bit_length() - 1)


def _mod(a, n):
    return a & (n - 1)


def _filled(buf, sem):
    pltpu.make_async_copy(buf, buf, sem).wait()


def _body(x_hbm, gw_hbm, k_hbm, v_hbm, wq_hbm, wo_hbm, wg_hbm, wu_hbm, wd_hbm, o_ref,
          kv_buf, wq_buf, wo_buf, wg_buf, wu_buf, wd_buf, x_buf, gw_buf, q_buf, h_buf, y_buf,
          kv_sem, w_sem, wd_sem):
    batch, d_model = x_buf.shape
    d_ff = wd_buf.shape[0]
    groups, _, d_head = q_buf.shape
    steps = k_hbm.shape[1] // TILE
    steps_per_head = steps // groups
    ff_blocks = h_buf.shape[0]
    ff_copies = d_ff // W_ROWS

    def rows(hbm, buf, piece, sem):
        r = pl.ds(pl.multiple_of(piece * W_ROWS, W_ROWS), W_ROWS)
        return pltpu.make_async_copy(hbm.at[r], buf.at[r], sem)

    def spread(a, s, queue):
        return (a * 2 + (s % 4) * 16 + s // 4) ^ (queue * 0x4A)

    def wq_piece(piece):
        cols = TILE * d_head // Q_ROWS
        per_row = wq_buf.shape[1] // cols
        r = pl.ds(pl.multiple_of(_div(piece, per_row) * Q_ROWS, Q_ROWS), Q_ROWS)
        c = pl.ds(pl.multiple_of(_mod(piece, per_row) * cols, cols), cols)
        return pltpu.make_async_copy(wq_hbm.at[r, c], wq_buf.at[r, c], w_sem.at[0])

    def start_kv(step, s):
        slot = _mod(step, RING)
        keys = pl.ds(pl.multiple_of(step * TILE, TILE), TILE)
        for queue, hbm in enumerate((k_hbm, v_hbm)):
            pltpu.make_async_copy(
                hbm.at[s, keys], kv_buf.at[slot, s, queue], kv_sem.at[slot]).start(priority=queue)

    x_copy = pltpu.make_async_copy(x_hbm, x_buf, w_sem.at[4])
    gw_copy = pltpu.make_async_copy(gw_hbm, gw_buf, w_sem.at[5])

    @pl.loop(0, 8)
    def _(a):
        for s in range(STREAMS):
            for queue in range(2):
                wq_piece(spread(a, s, queue)).start(priority=queue)

    x_copy.start()
    gw_copy.start()

    @pl.loop(0, 8)
    def _(a):
        for s in range(STREAMS):
            for queue in range(2):
                rows(wo_hbm, wo_buf, spread(a, s, queue), w_sem.at[1]).start(priority=queue)

    for lo, hi, n in ((0, ff_copies - 32, 3), (ff_copies - 32, 16, 2)):
        @pl.loop(lo, hi)
        def _(a):
            for j in range(n):
                rows(wg_hbm, wg_buf, j * 16 + a, w_sem.at[2]).start(priority=0)
                rows(wu_hbm, wu_buf, j * 16 + a, w_sem.at[3]).start(priority=1)

    @pl.loop(0, AHEAD)
    def _(step):
        for s in range(STREAMS):
            start_kv(step, s)

    for n, buf in enumerate((wq_buf, wo_buf, wg_buf, wu_buf)):
        _filled(buf, w_sem.at[n])
    x_copy.wait()
    gw_copy.wait()

    xf = x_buf[...].astype(jnp.float32)
    xf = jnp.concatenate([xf, xf], axis=0)
    x = xf.astype(jnp.bfloat16)
    gw = gw_buf[...].astype(jnp.float32)
    z = jnp.zeros((STREAMS, d_head), jnp.float32)
    for j in range(d_model // d_head):
        z += xf[:, j * d_head:(j + 1) * d_head] * gw[j:j + 1, :]
    gate = jax.nn.sigmoid(jnp.sum(z, axis=1, keepdims=True))

    row = lax.broadcasted_iota(jnp.int32, (STREAMS, TILE), 0)
    col = lax.broadcasted_iota(jnp.int32, (STREAMS, TILE), 1)
    zeros = jnp.zeros((STREAMS, TILE), jnp.float32)
    neg_inf = jnp.full((STREAMS, TILE), -jnp.inf, jnp.float32)

    def head(group, half):
        return pl.ds(pl.multiple_of((half * groups + group) * d_head, d_head), d_head)

    def project_q(group):
        q_buf[group] = jnp.where(row < batch,
                                 _dot(x, wq_buf[:, head(group, 0)]),
                                 _dot(x, wq_buf[:, head(group, 1)]))

    def project_out(group, l, acc):
        o = acc * (gate / jnp.sum(l, axis=1, keepdims=True))
        swapped = jnp.concatenate([o[batch:], o[:batch]], axis=0)
        y_buf[...] += (_dot(o.astype(jnp.bfloat16), wo_buf[head(group, 0), :])
                       + _dot(swapped.astype(jnp.bfloat16), wo_buf[head(group, 1), :]))

    def ffn_up(f):
        first = jnp.maximum(d_ff - (f + 1) * TILE, 0)
        r = pl.ds(pl.multiple_of(first, W_ROWS), TILE)
        g = _dot_t(x, wg_buf[r, :])
        u = _dot_t(x, wu_buf[r, :])
        h = g * jax.nn.sigmoid(g) * u * (1.0 - gate)
        h_buf[f] = jnp.where(first + col < d_ff - f * TILE, h, 0.0)

    def ffn_down(f):
        first = max(d_ff - (f + 1) * TILE, 0)
        return _dot(h_buf[f].astype(jnp.bfloat16), wd_buf[pl.ds(first, TILE), :])

    def attend(step, state, start_next, scores=True, values=True):
        s_prev, m, l, acc = state
        slot = _mod(step, RING)
        prev = _mod(step + RING - 1, RING)
        if scores:
            _filled(kv_buf.at[slot], kv_sem.at[slot])
            q = q_buf[_div(step, steps_per_head)].astype(jnp.bfloat16)
        if values:
            m_new = jnp.maximum(m, jnp.max(s_prev, axis=1, keepdims=True))
            alpha = jnp.exp(m - m_new)
            p = jnp.exp(s_prev - m_new)
            p_bf16 = p.astype(jnp.bfloat16)
        qk = pv = zeros
        for s in range(STREAMS):
            start_next(s)
            mine = row == (s % 2) * batch + s // 2
            if scores:
                qk = jnp.where(mine, _dot_t(q, kv_buf[slot, s, 0]), qk)
            if values:
                pv = jnp.where(mine, _dot(p_bf16, kv_buf[prev, s, 1]), pv)
        if values:
            m, l, acc = m_new, alpha * l + p, alpha * acc + pv
        return qk * d_head ** -0.5, m, l, acc

    y_buf[...] = jnp.zeros_like(y_buf)
    project_q(0)
    state = attend(0, (zeros, neg_inf, zeros, zeros), lambda s: start_kv(AHEAD, s), values=False)

    def attend_group(group, state):
        s_prev, _, l, acc = state

        @pl.when(group > 0)
        def _():
            project_out(group - 1, l, acc)

        @pl.when(group < ff_blocks)
        def _():
            ffn_up(group)

        @pl.when(group + 1 < groups)
        def _():
            project_q(group + 1)

        return lax.fori_loop(
            group * steps_per_head + 1,
            jnp.minimum((group + 1) * steps_per_head + 1, steps - AHEAD),
            lambda step, state: attend(step, state, lambda s: start_kv(step + AHEAD, s)),
            (s_prev, neg_inf, zeros, zeros))

    state = lax.fori_loop(0, groups, attend_group, state)

    per_step = ff_copies // AHEAD
    extra = ff_copies - per_step * AHEAD
    cuts = [d_ff - n * TILE for n in STAGES]
    for piece in range(extra):
        rows(wd_hbm, wd_buf, piece, wd_sem.at[0]).start(priority=1)

    def start_wd(j, s):
        if s < per_step:
            piece = extra + j * per_step + s
            stage = sum((piece >= cut // W_ROWS).astype(jnp.int32) for cut in cuts)
            rows(wd_hbm, wd_buf, piece, wd_sem.at[stage]).start(priority=1)

    state = lax.fori_loop(
        0, AHEAD,
        lambda j, state: attend(steps - AHEAD + j, state, lambda s: start_wd(j, s)), state)
    _, _, l, acc = attend(steps, state, lambda s: None, scores=False)
    project_out(groups - 1, l, acc)

    y = y_buf[...]
    edges = [0] + cuts + [d_ff]
    for stage, (lo, hi) in enumerate(zip(edges[:-1], edges[1:])):
        _filled(wd_buf.at[pl.ds(lo, hi - lo)], wd_sem.at[stage])
        for f in range((d_ff - hi) // TILE, pl.cdiv(d_ff - lo, TILE)):
            y += ffn_down(f)
    o_ref[...] = y[:batch].astype(o_ref.dtype)


def _kernel(*refs):
    pl.run_scoped(
        lambda *sems: _body(*refs, *sems),
        pltpu.SemaphoreType.DMA((RING,)),
        pltpu.SemaphoreType.DMA((6,)),
        pltpu.SemaphoreType.DMA((len(STAGES) + 1,)))


@jax.jit
def pallas_gated_mix__mha_block_cached__swiglu_ffn__decode_kernel(
    A_x: jax.Array,
    A_k_cache: jax.Array,
    A_v_cache: jax.Array,
    A_wq: jax.Array,
    A_wo: jax.Array,
    B_x: jax.Array,
    B_w_gate: jax.Array,
    B_w_up: jax.Array,
    B_w_down: jax.Array,
    gate_w: jax.Array,
):
    del B_x
    batch, q_len, d_model = A_x.shape
    _, heads, k_len, d_head = A_k_cache.shape
    d_ff = B_w_gate.shape[1]
    groups = batch * heads // STREAMS
    assert (2 * batch, q_len, d_head) == (STREAMS, 1, TILE)
    assert d_model * W_ROWS == TILE * d_head and heads * d_head == 128 * W_ROWS
    assert d_ff % W_ROWS == 0 and 32 <= d_ff // W_ROWS < STREAMS * AHEAD + AHEAD
    assert k_len & (k_len - 1) == 0 and k_len > AHEAD * TILE

    kv_shape = (STREAMS, groups * k_len, d_head)
    bf16, f32 = jnp.bfloat16, jnp.float32
    out = pl.pallas_call(
        _kernel,
        out_shape=jax.ShapeDtypeStruct((batch, d_model), A_x.dtype),
        in_specs=[pl.BlockSpec(memory_space=pl.ANY)] * 9,
        out_specs=pl.BlockSpec(memory_space=pltpu.VMEM),
        scratch_shapes=[
            pltpu.VMEM((RING, STREAMS, 2, TILE, d_head), bf16),
            pltpu.VMEM((d_model, heads * d_head), bf16),
            pltpu.VMEM((heads * d_head, d_model), bf16),
            pltpu.VMEM((d_ff, d_model), bf16),
            pltpu.VMEM((d_ff, d_model), bf16),
            pltpu.VMEM((d_ff, d_model), bf16),
            pltpu.VMEM((batch, d_model), bf16),
            pltpu.VMEM((d_model // d_head, d_head), bf16),
            pltpu.VMEM((groups, STREAMS, d_head), f32),
            pltpu.VMEM((pl.cdiv(d_ff, TILE), STREAMS, TILE), f32),
            pltpu.VMEM((STREAMS, d_model), f32),
        ],
        compiler_params=pltpu.CompilerParams(vmem_limit_bytes=32 * 2**20),
        name="gated_mix_decode",
    )(
        A_x.reshape(batch, d_model), gate_w.reshape(d_model // d_head, d_head),
        A_k_cache.reshape(kv_shape), A_v_cache.reshape(kv_shape),
        A_wq, A_wo, B_w_gate.T, B_w_up.T, B_w_down,
    )
    return out.reshape(batch, q_len, d_model)
```
